```python
import os as _os
_os.environ.setdefault("JAX_PLATFORMS", "cpu")
import jax
import jax.numpy as jnp

def _softmax(x, axis=-1):
    return jax.nn.softmax(x, axis=axis)
def _gelu(x):
    return jax.nn.gelu(x, approximate=True)
def _silu(x):
    return jax.nn.silu(x)
def _sigmoid(x):
    return jax.nn.sigmoid(x)
def _layernorm(x, axis=-1, eps=1e-5):
    m = jnp.mean(x, axis=axis, keepdims=True)
    v = jnp.var(x, axis=axis, keepdims=True)
    return (x - m) / jnp.sqrt(v + eps)
def _scatter_add(tgt, idx, src, axis=0):
    return tgt.at[idx].add(src)
def _segment_sum(src, seg, n):
    return jax.ops.segment_sum(src, seg, n)
class _Rng:
    def __init__(self, key):
        self._k = key
    def _next(self):
        self._k, sub = jax.random.split(self._k)
        return sub
    def normal(self, shape):
        return jax.random.normal(self._next(), shape, dtype=jnp.bfloat16)
    def randint(self, lo, hi, shape):
        return jax.random.randint(self._next(), shape, lo, hi, dtype=jnp.int32)
    def uniform(self, shape, lo=0.0, hi=1.0):
        return jax.random.uniform(self._next(), shape, jnp.bfloat16, lo, hi)
    def permutation(self, n):
        return jax.random.permutation(self._next(), n)


kernel_name = 'gated_mix__mha_block__mixer_s_mlp__prompt'

def setup_inputs():
    _rng = _Rng(jax.random.key(int.from_bytes(__import__("os").urandom(4), "little")))
    _w = (lambda a: (lambda t: t.astype(jnp.bfloat16) if jnp.issubdtype(t.dtype, jnp.floating) else t)(jnp.asarray(a)))
    def _A_setup():
        B, S, D, H = 1, 2048, 512, 32
        return {
            "x": _w((lambda *s: _rng.normal(s) * 0.05)(B, S, D)),
            "wqkv": _w((lambda *s: _rng.normal(s) * 0.8)(D, 3 * D)),
            "wo": _w((lambda *s: _rng.normal(s) * 0.05)(D, D)),
        }
    _A_in = _A_setup()

    def _B_setup():
        B, S, D, F = 1, 2048, 512, 1792
        return {
            "x":  _w((lambda *s: _rng.normal(s) * 0.05)(B, S, D)),
            "w1": _w((lambda *s: _rng.normal(s) * 0.2)(D, D) * (D ** -0.5)),
            "w2": _w((lambda *s: _rng.normal(s) * 0.2)(D, D) * (D ** -0.5)),
            "w3": _w((lambda *s: _rng.normal(s) * 0.2)(D, F) * (D ** -0.5)),
            "w4": _w((lambda *s: _rng.normal(s) * 0.2)(F, D) * (F ** -0.5)),
        }
    _B_in = _B_setup()

    return {
        "A_x": _A_in["x"],
        "A_wqkv": _A_in["wqkv"],
        "A_wo": _A_in["wo"],
        "B_x": _B_in["x"],
        "B_w1": _B_in["w1"],
        "B_w2": _B_in["w2"],
        "B_w3": _B_in["w3"],
        "B_w4": _B_in["w4"],
        "gate_w": _w((lambda *s: _rng.normal(s) * 0.05)(512) * 16.0),
    }

def reference(A_x, A_wqkv, A_wo, B_x, B_w1, B_w2, B_w3, B_w4, gate_w):
    def _A_ref(x, wqkv, wo):
        B, S, D = x.shape
        H = 32
        Dh = D // H
        qkv = (lambda x, *d: x.transpose(*d))((x @ wqkv).reshape(B, S, 3, H, Dh), 2, 0, 3, 1, 4)
        q, k, v = qkv[0], qkv[1], qkv[2]
        scores = jnp.einsum("bhqd,bhkd->bhqk", q, k) * (Dh ** -0.5)
        p = _softmax(scores, axis=-1)
        o = jnp.einsum("bhqk,bhkd->bhqd", p, v)
        return (lambda x, *d: x.transpose(*d))(o, 0, 2, 1, 3).reshape(B, S, D) @ wo

    def _B_ref(x, w1, w2, w3, w4):
        B, S, D = x.shape
        h = _gelu(_layernorm(x, axis=-1) @ w1)
        c = D // 4
        g0 = jnp.pad(h[:, :, 0*c:1*c], ((0, 0), (1, 0), (0, 0)))[:, :S, :]
        g1 = jnp.pad(h[:, :, 1*c:2*c], ((0, 0), (0, 1), (0, 0)))[:, 1:, :]
        g2 = jnp.pad(h[:, :, 2*c:3*c], ((0, 0), (2, 0), (0, 0)))[:, :S, :]
        g3 = jnp.pad(h[:, :, 3*c:   ], ((0, 0), (0, 2), (0, 0)))[:, 2:, :]
        hs = jnp.concatenate([g0, g1, g2, g3], axis=-1) @ w2
        x1 = x + hs
        h2 = _gelu(_layernorm(x1, axis=-1) @ w3) @ w4
        return x1 + h2

    x = A_x
    g = _sigmoid((x * gate_w).sum(-1, keepdims=True))
    a = _A_ref(x, A_wqkv, A_wo)
    b = _B_ref(x, B_w1, B_w2, B_w3, B_w4)
    return g * a + (1 - g) * b
```

```python
import jax
import jax.numpy as jnp
from jax import lax
import jax.experimental.pallas as pl
import jax.experimental.pallas.tpu as pltpu

S = 2048
D = 512
H = 32
DH = 16
F = 1792
TQ = 512
NQ = S // TQ
CH = 128
NC = S // CH
FC = 256
UNROLL = 8
PADR = 16
LOG2E = 1.4426950408889634
QSCALE = (DH ** -0.5) * LOG2E
L_LO = 2.0 ** -40
L_HI = 2.0 ** 40
O_HI = 3.0e38

F32 = jnp.float32
BF16 = jnp.bfloat16


def _dot(a, b):
    return jnp.dot(a, b, preferred_element_type=F32)


def _layernorm(x):
    m = jnp.mean(x, axis=-1, keepdims=True)
    xc = x - m
    v = jnp.mean(xc * xc, axis=-1, keepdims=True)
    return xc * lax.rsqrt(v + 1e-5)


def _gelu(x):
    return jax.nn.gelu(x, approximate=True)


def _kernel(xa_hbm, wqkv_hbm, wo_hbm, w1_hbm, w2_hbm, w3_hbm, w4_hbm, gw_hbm,
            o_ref,
            xa, wq, wk, wv, wo, w1, w2, w3, w4, gw_ref, sems,
            k4, qt, vt, x1buf, ln2buf, bbuf, oraw, p_a, p_b, lbuf, qp_a, qp_b):
    i = pl.program_id(0)

    copies = [(wqkv_hbm.at[:, pl.ds(D, D)], wk)]
    copies += [(xa_hbm.at[pl.ds(r * TQ, TQ), :], xa.at[pl.ds(PADR + r * TQ, TQ), :])
               for r in range(NQ)]
    copies += [(wqkv_hbm.at[:, pl.ds(0, D)], wq), (w1_hbm, w1),
               (wqkv_hbm.at[:, pl.ds(2 * D, D)], wv), (w2_hbm, w2),
               (w3_hbm, w3), (w4_hbm, w4), (wo_hbm, wo), (gw_hbm, gw_ref)]
    C_WK, C_X0, C_MIX, C_REST = 0, 1, 1 + NQ, 5 + NQ

    def copy(n):
        return pltpu.make_async_copy(copies[n][0], copies[n][1], sems.at[n])

    FLAG = 2 * H

    def normalise(u):
        row = pl.multiple_of((u % H) * DH, DH)
        l = jnp.sum(lbuf[u % (2 * H)], axis=0, keepdims=True)
        raw = oraw[pl.ds(row, DH), :]
        oraw[pl.ds(row, DH), :] = raw * (1.0 / l)
        amax = jnp.max(jnp.abs(raw).reshape(DH // 8, 8, TQ), axis=0)
        ok = (l >= L_LO) & (l <= L_HI) & (amax <= O_HI)
        lbuf[FLAG] = jnp.where(ok, lbuf[FLAG], 1.0)

    def pv_chunk(row, p_r, c):
        sl = slice(c * CH, (c + 1) * CH)
        return _dot(vt[pl.ds(row, DH), sl], p_r[sl, :])

    def stage_q(u, qp):
        un = jnp.minimum(u, NQ * H - 1)
        qp[pl.ds(pl.multiple_of(((u + 6) % 8) * DH, DH), DH), :] = jnp.zeros((DH, TQ), BF16)
        qp[pl.ds(pl.multiple_of((u % 8) * DH, DH), DH), :] = qt[
            pl.ds(pl.multiple_of((un % H) * DH, DH), DH),
            pl.ds(pl.multiple_of((un // H) * TQ, TQ), TQ)]

    def slot(u_a, p_w, u_b, p_r, u_c, qp_cur, qp_next):
        normalise(u_c)
        stage_q(u_a + 1, qp_next)
        g_a = (u_a % H) // 8
        row_b = pl.multiple_of((u_b % H) * DH, DH)
        acc = None
        lsum = None
        for c in range(NC):
            sl = slice(c * CH, (c + 1) * CH)
            p = jnp.exp2(_dot(k4[g_a, sl, :], qp_cur[...]))
            p_w[sl, :] = p.astype(BF16)
            ps = jnp.sum(p.reshape(CH // 8, 8, TQ), axis=0)
            lsum = ps if lsum is None else lsum + ps
            o = pv_chunk(row_b, p_r, c)
            acc = o if acc is None else acc + o
        lbuf[u_a % (2 * H)] = lsum
        oraw[pl.ds(row_b, DH), :] = acc

    def ln2_into(r):
        rs = pl.ds(pl.multiple_of(jnp.minimum(r, NQ - 1) * TQ, TQ), TQ)
        ln2buf[r % 2] = _layernorm(x1buf[rs, :]).astype(BF16)

    @pl.when(i == 0)
    def _prologue():
        copy(C_WK).start()
        copy(C_X0).start()
        copy(C_X0 + 1).start()
        xa[0:PADR, :] = jnp.zeros((PADR, D), BF16)
        xa[PADR + S:PADR + S + PADR, :] = jnp.zeros((PADR, D), BF16)
        lbuf[2 * H - 2:2 * H] = jnp.ones((2, 8, TQ), F32)
        oraw[D - 2 * DH:D, :] = jnp.zeros((2 * DH, TQ), F32)
        p_b[...] = jnp.zeros((S, TQ), BF16)
        copy(C_WK).wait()
        for n in range(C_X0 + 2, len(copies)):
            copy(n).start()

        def proj_k(r, carry):
            r0 = pl.multiple_of(r * TQ, TQ)
            xs = pl.ds(PADR + r0, TQ)
            pltpu.make_async_copy(xa_hbm.at[pl.ds(r0, TQ), :], xa.at[xs, :],
                                  sems.at[C_X0 + r]).wait()
            kk = _dot(xa[xs, :], wk[...]).astype(BF16)
            for g in range(4):
                k4[g, pl.ds(r0, TQ), :] = kk[:, g * 128:(g + 1) * 128]
            return carry

        lax.fori_loop(0, NQ, proj_k, 0)
        for n in range(C_MIX, C_REST):
            copy(n).wait()

        def proj_rest(r, carry):
            r0 = pl.multiple_of(r * TQ, TQ)
            rs = pl.ds(r0, TQ)
            x = xa[pl.ds(PADR + r0, TQ), :]
            qt[:, rs] = (_dot(x, wq[...]) * QSCALE).T.astype(BF16)
            xw = xa[pl.ds(r0, TQ + 2 * PADR), :].astype(F32)[8:TQ + 2 * PADR - 8]
            h = _gelu(_dot(_layernorm(xw).astype(BF16), w1[...]))
            vt[:, rs] = _dot(x, wv[...]).T.astype(BF16)
            c = D // 4
            hs_in = jnp.concatenate([
                h[8 - 1:8 - 1 + TQ, 0 * c:1 * c],
                h[8 + 1:8 + 1 + TQ, 1 * c:2 * c],
                h[8 - 2:8 - 2 + TQ, 2 * c:3 * c],
                h[8 + 2:8 + 2 + TQ, 3 * c:4 * c],
            ], axis=-1).astype(BF16)
            x1buf[rs, :] = x.astype(F32) + _dot(hs_in, w2[...])
            return carry

        lax.fori_loop(0, NQ, proj_rest, 0)
        ln2_into(0)
        qp_a[...] = jnp.zeros((128, TQ), BF16)
        qp_b[...] = jnp.zeros((128, TQ), BF16)
        stage_q(0, qp_a)
        for n in range(C_REST, len(copies)):
            copy(n).wait()

    lbuf[FLAG] = jnp.zeros((8, TQ), F32)
    u0 = i * H

    def body(j, carry):
        u = u0 + UNROLL * j
        for t in range(0, UNROLL, 2):
            slot(u + t, p_a, u + t + 2 * H - 1, p_b, u + t + 2 * H - 2, qp_a, qp_b)
            slot(u + t + 1, p_b, u + t, p_a, u + t + 2 * H - 1, qp_b, qp_a)
        return carry

    lax.fori_loop(0, H // UNROLL, body, 0)

    r0 = pl.multiple_of(i * TQ, TQ)
    logit = jnp.sum(xa[pl.ds(PADR + r0, TQ), :].astype(F32)
                    * gw_ref[...].astype(F32).reshape(1, D), axis=-1, keepdims=True)
    g = jax.nn.sigmoid(logit)

    def out_proj():
        return lax.dot_general(oraw[...].astype(BF16), wo[...], (((0,), (0,)), ((), ())),
                               preferred_element_type=F32)

    u_last = u0 + H - 1
    row_last = (H - 1) * DH
    pv = {"c": 0, "acc": None}

    def pv_chunks(n):
        for _ in range(n):
            c = pv["c"]
            if c == NC:
                return
            o = pv_chunk(row_last, p_b, c)
            pv["acc"] = o if pv["acc"] is None else pv["acc"] + o
            pv["c"] = c + 1
            if c + 1 == NC:
                oraw[row_last:row_last + DH, :] = pv["acc"]
                normalise(u_last)

    normalise(u_last - 1)
    x1 = x1buf[pl.ds(r0, TQ), :]
    nf = F // FC
    up = _dot(ln2buf[i % 2], w3[:, 0:FC])
    h2 = None
    part = None
    for f in range(nf):
        pv_chunks(2)
        act = _gelu(up).astype(BF16)
        if f + 1 < nf:
            up = _dot(ln2buf[i % 2], w3[:, (f + 1) * FC:(f + 2) * FC])
        pv_chunks(2)
        dn = _dot(act, w4[f * FC:(f + 1) * FC, :])
        h2 = dn if h2 is None else h2 + dn
        if f == 2:
            ln2_into(i + 1)
        if f == 4:
            part = g * out_proj()
    bb = x1 + h2
    bbuf[...] = bb
    o_ref[...] = (part + (1.0 - g) * bb).astype(o_ref.dtype)

    @pl.when(jnp.max(lbuf[FLAG]) > 0.0)
    def _exact():
        head_of_row = lax.broadcasted_iota(jnp.int32, (128, TQ), 0) // DH

        def ebody(h, carry):
            qg = qt[pl.ds(pl.multiple_of((h // 8) * 128, 128), 128), pl.ds(r0, TQ)]
            qpad = jnp.where(head_of_row == h % 8, qg, jnp.zeros_like(qg))
            s = _dot(k4[h // 8], qpad)
            m = jnp.max(s, axis=0, keepdims=True)
            p = jnp.exp2(s - m)
            l = jnp.sum(p, axis=0, keepdims=True)
            row = pl.multiple_of(h * DH, DH)
            o = _dot(vt[pl.ds(row, DH), :], p.astype(BF16))
            oraw[pl.ds(row, DH), :] = o * (1.0 / l)
            return carry

        lax.fori_loop(0, H, ebody, 0)
        o_ref[...] = (g * out_proj() + (1.0 - g) * bbuf[...]).astype(o_ref.dtype)


@jax.jit
def pallas_gated_mix__mha_block__mixer_s_mlp__prompt_kernel(
    A_x: jax.Array,
    A_wqkv: jax.Array,
    A_wo: jax.Array,
    B_x: jax.Array,
    B_w1: jax.Array,
    B_w2: jax.Array,
    B_w3: jax.Array,
    B_w4: jax.Array,
    gate_w: jax.Array,
):
    xa = A_x.reshape(S, D)
    del B_x

    any_spec = pl.BlockSpec(memory_space=pl.ANY)
    grid_spec = pltpu.PrefetchScalarGridSpec(
        num_scalar_prefetch=0,
        grid=(NQ,),
        in_specs=[any_spec] * 8,
        out_specs=pl.BlockSpec((TQ, D), lambda i: (i, 0)),
        scratch_shapes=[
            pltpu.VMEM((S + 2 * PADR, D), BF16),
            pltpu.VMEM((D, D), BF16),
            pltpu.VMEM((D, D), BF16),
            pltpu.VMEM((D, D), BF16),
            pltpu.VMEM((D, D), BF16),
            pltpu.VMEM((D, D), BF16),
            pltpu.VMEM((D, D), BF16),
            pltpu.VMEM((D, F), BF16),
            pltpu.VMEM((F, D), BF16),
            pltpu.VMEM((D,), BF16),
            pltpu.SemaphoreType.DMA((9 + NQ,)),
            pltpu.VMEM((4, S, 128), BF16),
            pltpu.VMEM((D, S), BF16),
            pltpu.VMEM((D, S), BF16),
            pltpu.VMEM((S, D), F32),
            pltpu.VMEM((2, TQ, D), BF16),
            pltpu.VMEM((TQ, D), F32),
            pltpu.VMEM((D, TQ), F32),
            pltpu.VMEM((S, TQ), BF16),
            pltpu.VMEM((S, TQ), BF16),
            pltpu.VMEM((2 * H + 1, 8, TQ), F32),
            pltpu.VMEM((128, TQ), BF16),
            pltpu.VMEM((128, TQ), BF16),
        ],
    )
    out = pl.pallas_call(
        _kernel,
        grid_spec=grid_spec,
        out_shape=jax.ShapeDtypeStruct((S, D), A_x.dtype),
        compiler_params=pltpu.CompilerParams(
            dimension_semantics=("arbitrary",),
            vmem_limit_bytes=100 * 1024 * 1024,
        ),
    )(xa, A_wqkv, A_wo, B_w1, B_w2, B_w3, B_w4, gate_w)
    return out.reshape(1, S, D)
```

```python
import jax
import jax.numpy as jnp
from jax import lax
import jax.experimental.pallas as pl
import jax.experimental.pallas.tpu as pltpu

S = 2048
D = 512
H = 32
DH = 16
F = 1792
TQ = 512
NQ = S // TQ
CH = 128
NC = S // CH
FC = 256
UNROLL = 8
PV_LAG = 2
PADR = 16
LOG2E = 1.4426950408889634
QSCALE = (DH ** -0.5) * LOG2E
L_LO = 2.0 ** -40
L_HI = 2.0 ** 40
O_HI = 3.0e38

F32 = jnp.float32
BF16 = jnp.bfloat16


def _dot(a, b):
    return jnp.dot(a, b, preferred_element_type=F32)


def _layernorm(x):
    m = jnp.mean(x, axis=-1, keepdims=True)
    xc = x - m
    v = jnp.mean(xc * xc, axis=-1, keepdims=True)
    return xc * lax.rsqrt(v + 1e-5)


def _gelu(x):
    return jax.nn.gelu(x, approximate=True)


def _kernel(xa_hbm, wqkv_hbm, wo_hbm, w1_hbm, w2_hbm, w3_hbm, w4_hbm, gw_hbm,
            o_ref,
            xa, wq, wk, wv, wo, w1, w2, w3, w4, gw_ref, sems,
            k4, qt, vt, x1buf, ln2buf, bbuf, oraw, p_a, p_b, lbuf, qp_a, qp_b):
    i = pl.program_id(0)

    copies = [(wqkv_hbm.at[:, pl.ds(D, D)], wk)]
    copies += [(xa_hbm.at[pl.ds(r * TQ, TQ), :], xa.at[pl.ds(PADR + r * TQ, TQ), :])
               for r in range(NQ)]
    copies += [(wqkv_hbm.at[:, pl.ds(0, D)], wq), (w1_hbm, w1),
               (wqkv_hbm.at[:, pl.ds(2 * D, D)], wv), (w2_hbm, w2),
               (w3_hbm, w3), (w4_hbm, w4), (wo_hbm, wo), (gw_hbm, gw_ref)]
    C_WK, C_X0, C_MIX, C_REST = 0, 1, 1 + NQ, 5 + NQ

    def copy(n):
        return pltpu.make_async_copy(copies[n][0], copies[n][1], sems.at[n])

    FLAG = 2 * H

    def normalise(u):
        row = pl.multiple_of((u % H) * DH, DH)
        l = jnp.sum(lbuf[u % (2 * H)], axis=0, keepdims=True)
        raw = oraw[pl.ds(row, DH), :]
        oraw[pl.ds(row, DH), :] = raw * (1.0 / l)
        amax = jnp.max(jnp.abs(raw).reshape(DH // 8, 8, TQ), axis=0)
        ok = (l >= L_LO) & (l <= L_HI) & (amax <= O_HI)
        lbuf[FLAG] = jnp.where(ok, lbuf[FLAG], 1.0)

    def pv_chunk(row, p_r, c):
        sl = slice(c * CH, (c + 1) * CH)
        return _dot(vt[pl.ds(row, DH), sl], p_r[sl, :])

    def stage_q(u, qp):
        un = jnp.minimum(u, NQ * H - 1)
        qp[pl.ds(pl.multiple_of(((u + 6) % 8) * DH, DH), DH), :] = jnp.zeros((DH, TQ), BF16)
        qp[pl.ds(pl.multiple_of((u % 8) * DH, DH), DH), :] = qt[
            pl.ds(pl.multiple_of((un % H) * DH, DH), DH),
            pl.ds(pl.multiple_of((un // H) * TQ, TQ), TQ)]

    def slot(u_a, p_w, u_b, p_r, u_c, qp_cur, qp_next):
        normalise(u_c)
        stage_q(u_a + 1, qp_next)
        g_a = (u_a % H) // 8
        row_b = pl.multiple_of((u_b % H) * DH, DH)
        acc = None
        lsum = None
        for c in range(NC + PV_LAG):
            if c < NC:
                sl = slice(c * CH, (c + 1) * CH)
                p = jnp.exp2(_dot(k4[g_a, sl, :], qp_cur[...]))
                p_w[sl, :] = p.astype(BF16)
                ps = jnp.sum(p.reshape(CH // 8, 8, TQ), axis=0)
                lsum = ps if lsum is None else lsum + ps
            if c >= PV_LAG:
                o = pv_chunk(row_b, p_r, c - PV_LAG)
                acc = o if acc is None else acc + o
        lbuf[u_a % (2 * H)] = lsum
        oraw[pl.ds(row_b, DH), :] = acc

    def ln2_into(r):
        rs = pl.ds(pl.multiple_of(jnp.minimum(r, NQ - 1) * TQ, TQ), TQ)
        ln2buf[r % 2] = _layernorm(x1buf[rs, :]).astype(BF16)

    @pl.when(i == 0)
    def _prologue():
        copy(C_WK).start()
        copy(C_X0).start()
        copy(C_X0 + 1).start()
        xa[0:PADR, :] = jnp.zeros((PADR, D), BF16)
        xa[PADR + S:PADR + S + PADR, :] = jnp.zeros((PADR, D), BF16)
        lbuf[2 * H - 2:2 * H] = jnp.ones((2, 8, TQ), F32)
        oraw[D - 2 * DH:D, :] = jnp.zeros((2 * DH, TQ), F32)
        p_b[...] = jnp.zeros((S, TQ), BF16)
        copy(C_WK).wait()
        for n in range(C_X0 + 2, len(copies)):
            copy(n).start()

        def proj_k(r, carry):
            r0 = pl.multiple_of(r * TQ, TQ)
            xs = pl.ds(PADR + r0, TQ)
            pltpu.make_async_copy(xa_hbm.at[pl.ds(r0, TQ), :], xa.at[xs, :],
                                  sems.at[C_X0 + r]).wait()
            kk = _dot(xa[xs, :], wk[...]).astype(BF16)
            for g in range(4):
                k4[g, pl.ds(r0, TQ), :] = kk[:, g * 128:(g + 1) * 128]
            return carry

        lax.fori_loop(0, NQ, proj_k, 0)
        for n in range(C_MIX, C_REST):
            copy(n).wait()

        def proj_rest(r, carry):
            r0 = pl.multiple_of(r * TQ, TQ)
            rs = pl.ds(r0, TQ)
            x = xa[pl.ds(PADR + r0, TQ), :]
            qt[:, rs] = (_dot(x, wq[...]) * QSCALE).T.astype(BF16)
            xw = xa[pl.ds(r0, TQ + 2 * PADR), :].astype(F32)[8:TQ + 2 * PADR - 8]
            h = _gelu(_dot(_layernorm(xw).astype(BF16), w1[...]))
            vt[:, rs] = _dot(x, wv[...]).T.astype(BF16)
            c = D // 4
            hs_in = jnp.concatenate([
                h[8 - 1:8 - 1 + TQ, 0 * c:1 * c],
                h[8 + 1:8 + 1 + TQ, 1 * c:2 * c],
                h[8 - 2:8 - 2 + TQ, 2 * c:3 * c],
                h[8 + 2:8 + 2 + TQ, 3 * c:4 * c],
            ], axis=-1).astype(BF16)
            x1buf[rs, :] = x.astype(F32) + _dot(hs_in, w2[...])
            return carry

        lax.fori_loop(0, NQ, proj_rest, 0)
        ln2_into(0)
        qp_a[...] = jnp.zeros((128, TQ), BF16)
        qp_b[...] = jnp.zeros((128, TQ), BF16)
        stage_q(0, qp_a)
        for n in range(C_REST, len(copies)):
            copy(n).wait()

    lbuf[FLAG] = jnp.zeros((8, TQ), F32)
    u0 = i * H

    def body(j, carry):
        u = u0 + UNROLL * j
        for t in range(0, UNROLL, 2):
            slot(u + t, p_a, u + t + 2 * H - 1, p_b, u + t + 2 * H - 2, qp_a, qp_b)
            slot(u + t + 1, p_b, u + t, p_a, u + t + 2 * H - 1, qp_b, qp_a)
        return carry

    lax.fori_loop(0, H // UNROLL, body, 0)

    r0 = pl.multiple_of(i * TQ, TQ)
    logit = jnp.sum(xa[pl.ds(PADR + r0, TQ), :].astype(F32)
                    * gw_ref[...].astype(F32).reshape(1, D), axis=-1, keepdims=True)
    g = jax.nn.sigmoid(logit)

    def out_proj():
        return lax.dot_general(oraw[...].astype(BF16), wo[...], (((0,), (0,)), ((), ())),
                               preferred_element_type=F32)

    u_last = u0 + H - 1
    row_last = (H - 1) * DH
    pv = {"c": 0, "acc": None}

    def pv_chunks(n):
        for _ in range(n):
            c = pv["c"]
            if c == NC:
                return
            o = pv_chunk(row_last, p_b, c)
            pv["acc"] = o if pv["acc"] is None else pv["acc"] + o
            pv["c"] = c + 1
            if c + 1 == NC:
                oraw[row_last:row_last + DH, :] = pv["acc"]
                normalise(u_last)

    normalise(u_last - 1)
    x1 = x1buf[pl.ds(r0, TQ), :]
    nf = F // FC
    up = _dot(ln2buf[i % 2], w3[:, 0:FC])
    h2 = None
    part = None
    for f in range(nf):
        pv_chunks(2)
        act = _gelu(up).astype(BF16)
        if f + 1 < nf:
            up = _dot(ln2buf[i % 2], w3[:, (f + 1) * FC:(f + 2) * FC])
        pv_chunks(2)
        dn = _dot(act, w4[f * FC:(f + 1) * FC, :])
        h2 = dn if h2 is None else h2 + dn
        if f == 2:
            ln2_into(i + 1)
        if f == 4:
            part = g * out_proj()
    bb = x1 + h2
    bbuf[...] = bb
    o_ref[...] = (part + (1.0 - g) * bb).astype(o_ref.dtype)

    @pl.when(jnp.max(lbuf[FLAG]) > 0.0)
    def _exact():
        head_of_row = lax.broadcasted_iota(jnp.int32, (128, TQ), 0) // DH

        def ebody(h, carry):
            qg = qt[pl.ds(pl.multiple_of((h // 8) * 128, 128), 128), pl.ds(r0, TQ)]
            qpad = jnp.where(head_of_row == h % 8, qg, jnp.zeros_like(qg))
            s = _dot(k4[h // 8], qpad)
            m = jnp.max(s, axis=0, keepdims=True)
            p = jnp.exp2(s - m)
            l = jnp.sum(p, axis=0, keepdims=True)
            row = pl.multiple_of(h * DH, DH)
            o = _dot(vt[pl.ds(row, DH), :], p.astype(BF16))
            oraw[pl.ds(row, DH), :] = o * (1.0 / l)
            return carry

        lax.fori_loop(0, H, ebody, 0)
        o_ref[...] = (g * out_proj() + (1.0 - g) * bbuf[...]).astype(o_ref.dtype)


@jax.jit
def pallas_gated_mix__mha_block__mixer_s_mlp__prompt_kernel(
    A_x: jax.Array,
    A_wqkv: jax.Array,
    A_wo: jax.Array,
    B_x: jax.Array,
    B_w1: jax.Array,
    B_w2: jax.Array,
    B_w3: jax.Array,
    B_w4: jax.Array,
    gate_w: jax.Array,
):
    xa = A_x.reshape(S, D)
    del B_x

    any_spec = pl.BlockSpec(memory_space=pl.ANY)
    grid_spec = pltpu.PrefetchScalarGridSpec(
        num_scalar_prefetch=0,
        grid=(NQ,),
        in_specs=[any_spec] * 8,
        out_specs=pl.BlockSpec((TQ, D), lambda i: (i, 0)),
        scratch_shapes=[
            pltpu.VMEM((S + 2 * PADR, D), BF16),
            pltpu.VMEM((D, D), BF16),
            pltpu.VMEM((D, D), BF16),
            pltpu.VMEM((D, D), BF16),
            pltpu.VMEM((D, D), BF16),
            pltpu.VMEM((D, D), BF16),
            pltpu.VMEM((D, D), BF16),
            pltpu.VMEM((D, F), BF16),
            pltpu.VMEM((F, D), BF16),
            pltpu.VMEM((D,), BF16),
            pltpu.SemaphoreType.DMA((9 + NQ,)),
            pltpu.VMEM((4, S, 128), BF16),
            pltpu.VMEM((D, S), BF16),
            pltpu.VMEM((D, S), BF16),
            pltpu.VMEM((S, D), F32),
            pltpu.VMEM((2, TQ, D), BF16),
            pltpu.VMEM((TQ, D), F32),
            pltpu.VMEM((D, TQ), F32),
            pltpu.VMEM((S, TQ), BF16),
            pltpu.VMEM((S, TQ), BF16),
            pltpu.VMEM((2 * H + 1, 8, TQ), F32),
            pltpu.VMEM((128, TQ), BF16),
            pltpu.VMEM((128, TQ), BF16),
        ],
    )
    out = pl.pallas_call(
        _kernel,
        grid_spec=grid_spec,
        out_shape=jax.ShapeDtypeStruct((S, D), A_x.dtype),
        compiler_params=pltpu.CompilerParams(
            dimension_semantics=("arbitrary",),
            vmem_limit_bytes=100 * 1024 * 1024,
        ),
    )(xa, A_wqkv, A_wo, B_w1, B_w2, B_w3, B_w4, gate_w)
    return out.reshape(1, S, D)
```
